```python
import os as _os
_os.environ.setdefault("JAX_PLATFORMS", "cpu")
import jax
import jax.numpy as jnp

def _softmax(x, axis=-1):
    return jax.nn.softmax(x, axis=axis)
def _gelu(x):
    return jax.nn.gelu(x, approximate=True)
def _silu(x):
    return jax.nn.silu(x)
def _sigmoid(x):
    return jax.nn.sigmoid(x)
def _layernorm(x, axis=-1, eps=1e-5):
    m = jnp.mean(x, axis=axis, keepdims=True)
    v = jnp.var(x, axis=axis, keepdims=True)
    return (x - m) / jnp.sqrt(v + eps)
def _scatter_add(tgt, idx, src, axis=0):
    return tgt.at[idx].add(src)
def _segment_sum(src, seg, n):
    return jax.ops.segment_sum(src, seg, n)
class _Rng:
    def __init__(self, key):
        self._k = key
    def _next(self):
        self._k, sub = jax.random.split(self._k)
        return sub
    def normal(self, shape):
        return jax.random.normal(self._next(), shape, dtype=jnp.bfloat16)
    def randint(self, lo, hi, shape):
        return jax.random.randint(self._next(), shape, lo, hi, dtype=jnp.int32)
    def uniform(self, shape, lo=0.0, hi=1.0):
        return jax.random.uniform(self._next(), shape, jnp.bfloat16, lo, hi)
    def permutation(self, n):
        return jax.random.permutation(self._next(), n)


kernel_name = 'recurrent_scan__ssm_conv_s5__mixer_s_mlp__prompt'

def setup_inputs():
    _rng = _Rng(jax.random.key(int.from_bytes(__import__("os").urandom(4), "little")))
    _w = (lambda a: (lambda t: t.astype(jnp.bfloat16) if jnp.issubdtype(t.dtype, jnp.floating) else t)(jnp.asarray(a)))
    def _A_setup():
        B, S, D = 1, 2048, 640
        P = D
        Lambda_re = -0.5 * jnp.exp((lambda *s: _rng.normal(s) * 0.8)(P))
        Lambda_im = (lambda *s: _rng.normal(s) * 0.8)(P) * 1.0
        B_re = (lambda *s: _rng.normal(s) * 0.8)(P, D) * (D ** -0.5)
        B_im = (lambda *s: _rng.normal(s) * 0.8)(P, D) * (D ** -0.5)
        C_re = (lambda *s: _rng.normal(s) * 0.8)(D, P) * (P ** -0.5)
        C_im = (lambda *s: _rng.normal(s) * 0.8)(D, P) * (P ** -0.5)
        log_dt = (lambda *s: _rng.normal(s) * 0.8)(P) * 0.3 - 2.0
        Dskip = (lambda *s: _rng.normal(s) * 0.8)(D)
        return {
            "x": _w((lambda *s: _rng.normal(s) * 0.05)(B, S, D)),
            "Lambda_re": _w(Lambda_re),
            "Lambda_im": _w(Lambda_im),
            "B_re": _w(B_re),
            "B_im": _w(B_im),
            "C_re": _w(C_re),
            "C_im": _w(C_im),
            "log_dt": _w(log_dt),
            "Dskip": _w(Dskip),
        }
    _A_in = _A_setup()

    def _B_setup():
        B, S, D, F = 1, 2048, 640, 1536
        return {
            "x":  _w((lambda *s: _rng.normal(s) * 0.05)(B, S, D)),
            "w1": _w((lambda *s: _rng.normal(s) * 0.8)(D, D) * (D ** -0.5)),
            "w2": _w((lambda *s: _rng.normal(s) * 0.8)(D, D) * (D ** -0.5)),
            "w3": _w((lambda *s: _rng.normal(s) * 0.8)(D, F) * (D ** -0.5)),
            "w4": _w((lambda *s: _rng.normal(s) * 0.8)(F, D) * (F ** -0.5)),
        }
    _B_in = _B_setup()

    return {
        "A_x": _A_in["x"],
        "A_Lambda_re": _A_in["Lambda_re"],
        "A_Lambda_im": _A_in["Lambda_im"],
        "A_B_re": _A_in["B_re"],
        "A_B_im": _A_in["B_im"],
        "A_C_re": _A_in["C_re"],
        "A_C_im": _A_in["C_im"],
        "A_log_dt": _A_in["log_dt"],
        "A_Dskip": _A_in["Dskip"],
        "B_x": _B_in["x"],
        "B_w1": _B_in["w1"],
        "B_w2": _B_in["w2"],
        "B_w3": _B_in["w3"],
        "B_w4": _B_in["w4"],
    }

def reference(A_x, A_Lambda_re, A_Lambda_im, A_B_re, A_B_im, A_C_re, A_C_im, A_log_dt, A_Dskip, B_x, B_w1, B_w2, B_w3, B_w4):
    def _A_ref(x, Lambda_re, Lambda_im, B_re, B_im, C_re, C_im, log_dt, Dskip):
        Bsz, L, H = x.shape
        Lam = Lambda_re + 1j * Lambda_im
        Bmat = B_re + 1j * B_im
        Cmat = C_re + 1j * C_im
        dt = jnp.exp(log_dt)
        Lam_bar = jnp.exp(dt * Lam)
        B_bar = ((Lam_bar - 1.0) / Lam)[:, None] * Bmat
        Bu = jnp.einsum("bld,pd->blp", x + 0j, B_bar)
        h = jnp.zeros_like(Bu[:, 0, :])
        hs = []
        for t in range(L):
            h = Lam_bar[None, :] * h + Bu[:, t, :]
            hs.append(h)
        hseq = jnp.stack(hs, 1)
        y = 2.0 * jnp.einsum("blp,dp->bld", hseq, Cmat).real + x * Dskip[None, None, :]
        return y

    def _B_ref(x, w1, w2, w3, w4):
        B, S, D = x.shape
        h = _gelu(_layernorm(x, axis=-1) @ w1)
        c = D // 4
        g0 = jnp.pad(h[:, :, 0*c:1*c], ((0, 0), (1, 0), (0, 0)))[:, :S, :]
        g1 = jnp.pad(h[:, :, 1*c:2*c], ((0, 0), (0, 1), (0, 0)))[:, 1:, :]
        g2 = jnp.pad(h[:, :, 2*c:3*c], ((0, 0), (2, 0), (0, 0)))[:, :S, :]
        g3 = jnp.pad(h[:, :, 3*c:   ], ((0, 0), (0, 2), (0, 0)))[:, 2:, :]
        hs = jnp.concatenate([g0, g1, g2, g3], axis=-1) @ w2
        x1 = x + hs
        h2 = _gelu(_layernorm(x1, axis=-1) @ w3) @ w4
        return x1 + h2

    x = A_x
    xn = _layernorm(x, axis=-1)
    s = _A_ref(xn, A_Lambda_re, A_Lambda_im, A_B_re, A_B_im, A_C_re, A_C_im, A_log_dt, A_Dskip)
    g = _silu(_B_ref(xn, B_w1, B_w2, B_w3, B_w4))
    return x + s * g
```

```python
import functools
import jax
import jax.numpy as jnp
from jax import lax
import jax.experimental.pallas as pl
import jax.experimental.pallas.tpu as pltpu

F32 = jnp.float32
BF16 = jnp.bfloat16
NT_DIMS = (((1,), (1,)), ((), ()))
NSEG = 8
HALO = 16
RC = 32


def _ln(v):
    m = jnp.mean(v, axis=-1, keepdims=True)
    d = v - m
    var = jnp.mean(d * d, axis=-1, keepdims=True)
    return d * lax.rsqrt(var + 1e-5)


def _gelu(v):
    return jax.nn.gelu(v, approximate=True)


def _t8(vs):
    vs = list(vs)
    sub = lax.broadcasted_iota(jnp.int32, vs[0].shape, 0)
    for d in (4, 2, 1):
        m = (sub & d) != 0
        for a in range(8):
            if a & d:
                continue
            A, B = vs[a], vs[a + d]
            vs[a] = jnp.where(m, pltpu.roll(B, d, 0), A)
            vs[a + d] = jnp.where(m, B, pltpu.roll(A, 8 - d, 0))
    return vs


def _kernel(x_hbm, lre_ref, lim_ref, ldt_ref, dsk_ref,
            bre_hbm, bim_hbm, cre_hbm, cim_hbm, w1_hbm, w2_hbm, w3_hbm, w4_hbm,
            o_hbm,
            xv, bre, bim, cre, cim, w1, w2, w3, w4,
            cp_ref, a_ref, lx_ref, bu_ref, hb_ref, carry_ref, hext_ref, xs_ref, xp_ref,
            ys_ref, x1_ref, xd_ref, sems, obuf, osems, *, T, L, D):
    P = D
    S = T // NSEG
    NC = P // 128
    NTL = L // T

    wpairs = [(bre_hbm, bre), (bim_hbm, bim), (w1_hbm, w1), (w2_hbm, w2),
              (cre_hbm, cre), (cim_hbm, cim), (w3_hbm, w3), (w4_hbm, w4)]

    def wcopy(k):
        return pltpu.make_async_copy(wpairs[k][0], wpairs[k][1], sems.at[k])

    def xcopy(k):
        return pltpu.make_async_copy(x_hbm.at[pl.ds(k * T, T)], xv.at[pl.ds(k * T, T)],
                                     sems.at[8 + k])

    def ocopy(t):
        slot = lax.rem(t, 2)
        return pltpu.make_async_copy(obuf.at[slot], o_hbm.at[pl.ds(t * T, T)], osems.at[slot])

    def vec(r):
        return r[...].astype(F32).reshape(1, D)

    def lam_terms():
        lre = vec(lre_ref)
        lim = vec(lim_ref)
        dt = jnp.exp(vec(ldt_ref)).astype(BF16).astype(F32)
        zr = dt * lre
        zi = dt * lim
        mag = jnp.exp(zr)
        ar = mag * jnp.cos(zi)
        ai = mag * jnp.sin(zi)
        return lre, lim, ar, ai

    def init_tables():
        _, _, ar, ai = lam_terms()
        ar8 = jnp.broadcast_to(ar, (8, P))
        ai8 = jnp.broadcast_to(ai, (8, P))
        a_ref[0:8, 0:P] = ar8
        a_ref[0:8, P:2 * P] = ai8
        pr, pi = ar8, ai8
        k = 1
        while k < S:
            pr, pi = pr * pr - pi * pi, 2.0 * pr * pi
            k *= 2
        a_ref[8:16, 0:P] = pr
        a_ref[8:16, P:2 * P] = pi
        carry_ref[...] = jnp.zeros(carry_ref.shape, F32)
        hext_ref[0:8, :] = jnp.zeros((8, D), F32)

    def init_c():
        lre, lim, ar, ai = lam_terms()
        nr = ar - 1.0
        ni = ai
        den = lre * lre + lim * lim
        cr = (nr * lre + ni * lim) / den
        ci = (ni * lre - nr * lim) / den
        crev = cre[...].astype(F32)
        cimv = cim[...].astype(F32)
        cp_ref[:, 0:P] = (2.0 * (crev * cr - cimv * ci)).astype(BF16)
        cp_ref[:, P:2 * P] = (-2.0 * (crev * ci + cimv * cr)).astype(BF16)

    def stage_a0(t):
        r0 = pl.multiple_of(t * T, T)
        nstart = pl.multiple_of(jnp.minimum(r0 + T, L - HALO), HALO)
        for cidx in range(T // RC):
            xc = xv[pl.ds(r0 + cidx * RC, RC), :].astype(F32)
            xnc = _ln(xc).astype(BF16).astype(F32)
            xs_ref[cidx * RC:(cidx + 1) * RC, :] = xnc
            lx_ref[cidx * RC:(cidx + 1) * RC, :] = _ln(xnc).astype(BF16)
        xh = xv[pl.ds(nstart, HALO), :].astype(F32)
        xnhf = _ln(xh).astype(BF16).astype(F32)
        lx_ref[T:T + HALO, :] = _ln(xnhf).astype(BF16)
        for q in range(S // 8):
            for j in range(NC):
                cs = slice(128 * j, 128 * (j + 1))
                w = _t8([xs_ref[seg * S + 8 * q:seg * S + 8 * q + 8, cs] for seg in range(NSEG)])
                for k2 in range(4):
                    r = (8 * q + 2 * k2) * 8
                    xp_ref[r:r + 16, cs] = jnp.concatenate(
                        [w[2 * k2], w[2 * k2 + 1]], axis=0).astype(BF16)

    def f1(t, first):
        if first:
            wcopy(0).wait()
            wcopy(1).wait()
        xp = xp_ref[...]
        bu_ref[:, 0:P] = lax.dot_general(xp, bre[...], NT_DIMS, preferred_element_type=F32)
        bu_ref[:, P:2 * P] = lax.dot_general(xp, bim[...], NT_DIMS, preferred_element_type=F32)
        if first:
            wcopy(2).wait()
        h = _gelu(jnp.dot(lx_ref[...], w1[...], preferred_element_type=F32))
        hext_ref[8:8 + T, :] = h[0:T]
        hext_ref[8 + T:8 + T + HALO, :] = jnp.where(t < NTL - 1, h[T:T + HALO], 0.0)

    def f2():
        sub = lax.broadcasted_iota(jnp.int32, (NSEG, 128), 0)
        for j in range(NC):
            cs = slice(128 * j, 128 * (j + 1))
            ci_ = slice(P + 128 * j, P + 128 * (j + 1))
            ar8 = a_ref[0:8, cs]
            ai8 = a_ref[0:8, ci_]
            hr = bu_ref[0:8, cs]
            hi = bu_ref[0:8, ci_]
            for s in range(1, S):
                rs = slice(8 * s, 8 * (s + 1))
                br = bu_ref[rs, cs]
                bi = bu_ref[rs, ci_]
                hr, hi = ar8 * hr - ai8 * hi + br, ar8 * hi + ai8 * hr + bi
            asr = a_ref[8:9, cs]
            asi = a_ref[8:9, ci_]
            cr = carry_ref[0:1, cs]
            ci = carry_ref[0:1, ci_]
            c8r = jnp.zeros((NSEG, 128), F32)
            c8i = jnp.zeros((NSEG, 128), F32)
            for q in range(NSEG):
                c8r = jnp.where(sub == q, cr, c8r)
                c8i = jnp.where(sub == q, ci, c8i)
                cr, ci = (asr * cr - asi * ci + hr[q:q + 1, :],
                          asr * ci + asi * cr + hi[q:q + 1, :])
            carry_ref[0:1, cs] = cr
            carry_ref[0:1, ci_] = ci
            hr, hi = c8r, c8i
            for s2 in range(S // 2):
                prs, pis = [], []
                for s in (2 * s2, 2 * s2 + 1):
                    rs = slice(8 * s, 8 * (s + 1))
                    br = bu_ref[rs, cs]
                    bi = bu_ref[rs, ci_]
                    hr, hi = ar8 * hr - ai8 * hi + br, ar8 * hi + ai8 * hr + bi
                    prs.append(hr)
                    pis.append(hi)
                rs = slice(16 * s2, 16 * (s2 + 1))
                hb_ref[rs, cs] = jnp.concatenate(prs, axis=0).astype(BF16)
                hb_ref[rs, ci_] = jnp.concatenate(pis, axis=0).astype(BF16)

    def f3(t, first):
        slot = lax.rem(t, 2)
        c = D // 4
        shifts = (-1, 1, -2, 2)
        cols = []
        for j in range(D // 128):
            lo, hi_ = 128 * j, 128 * (j + 1)
            g_lo, g_hi = lo // c, (hi_ - 1) // c
            a = hext_ref[pl.ds(8 + shifts[g_lo], T), lo:hi_]
            if g_hi != g_lo:
                b = hext_ref[pl.ds(8 + shifts[g_hi], T), lo:hi_]
                lane = lax.broadcasted_iota(jnp.int32, (T, 128), 1) + lo
                a = jnp.where(lane < g_hi * c, a, b)
            cols.append(a.astype(BF16))
        hsft = jnp.concatenate(cols, axis=1)
        hext_ref[0:8, :] = hext_ref[T:T + 8, :]
        if first:
            wcopy(3).wait()
        xn2 = xs_ref[...]
        x1_ref[slot] = xn2 + jnp.dot(hsft, w2[...], preferred_element_type=F32)
        xd_ref[slot] = xn2 * vec(dsk_ref)
        if first:
            xcopy(2).wait()
            stage_a0(1)
            wcopy(4).wait()
            wcopy(5).wait()
            xcopy(3).wait()
            init_c()
        ys_ref[slot] = lax.dot_general(hb_ref[...], cp_ref[...], NT_DIMS,
                                       preferred_element_type=F32)
        if not first:
            stage_a0(jnp.minimum(t + 1, NTL - 1))

    def b1(t):
        slot = lax.rem(t, 2)
        l1 = _ln(x1_ref[slot]).astype(BF16)
        return _gelu(jnp.dot(l1, w3[...], preferred_element_type=F32)).astype(BF16)

    def b2(t, u):
        slot = lax.rem(t, 2)
        h2 = jnp.dot(u, w4[...], preferred_element_type=F32)
        z = x1_ref[slot] + h2
        g = z * jax.nn.sigmoid(z)
        ycols = []
        for j in range(NC):
            cs = slice(128 * j, 128 * (j + 1))
            rows = [None] * (T // 8)
            for q in range(S // 8):
                w = _t8([ys_ref[slot, (8 * q + k) * 8:(8 * q + k) * 8 + 8, cs] for k in range(8)])
                for seg in range(NSEG):
                    rows[seg * (S // 8) + q] = w[seg]
            ycols.append(jnp.concatenate(rows, axis=0))
        sval = jnp.concatenate(ycols, axis=1) + xd_ref[slot]
        rp = pl.multiple_of(t * T, T)
        obuf[slot] = xv[pl.ds(rp, T), :].astype(F32) + sval * g

    xcopy(0).start()
    xcopy(1).start()
    for k in range(3):
        wcopy(k).start()
    xcopy(2).start()
    for k in range(3, 6):
        wcopy(k).start()
    xcopy(3).start()
    wcopy(6).start()
    wcopy(7).start()
    for k in range(4, NTL):
        xcopy(k).start()
    init_tables()
    xcopy(0).wait()
    xcopy(1).wait()
    stage_a0(0)
    f1(0, True)
    f2()
    f3(0, True)
    f1(1, False)
    f2()
    f3(1, False)
    wcopy(6).wait()
    wcopy(7).wait()

    def loop(i, carry):
        @pl.when(i + 2 < NTL)
        def _():
            xcopy(i + 2).wait()

        @pl.when(i >= 4)
        def _():
            ocopy(i - 4).wait()

        f1(i, False)
        u = b1(i - 2)
        f2()
        b2(i - 2, u)
        f3(i, False)
        ocopy(i - 2).start()
        return carry

    lax.fori_loop(2, NTL, loop, 0)

    ocopy(NTL - 4).wait()
    ocopy(NTL - 3).wait()
    u0 = b1(NTL - 2)
    u1 = b1(NTL - 1)
    b2(NTL - 2, u0)
    ocopy(NTL - 2).start()
    b2(NTL - 1, u1)
    ocopy(NTL - 1).start()
    ocopy(NTL - 2).wait()
    ocopy(NTL - 1).wait()


def _run(A_x, A_Lambda_re, A_Lambda_im, A_B_re, A_B_im, A_C_re, A_C_im, A_log_dt,
         A_Dskip, B_w1, B_w2, B_w3, B_w4, T=256):
    _, L, D = A_x.shape
    Fd = B_w3.shape[1]
    NTL = L // T
    x2 = A_x.reshape(L, D)
    anyspec = pl.BlockSpec(memory_space=pl.ANY)
    vspec = pl.BlockSpec(memory_space=pltpu.VMEM)
    out = pl.pallas_call(
        functools.partial(_kernel, T=T, L=L, D=D),
        in_specs=[anyspec, vspec, vspec, vspec, vspec] + [anyspec] * 8,
        out_specs=anyspec,
        out_shape=jax.ShapeDtypeStruct((L, D), F32),
        scratch_shapes=[
            pltpu.VMEM((L, D), BF16),
            pltpu.VMEM((D, D), BF16), pltpu.VMEM((D, D), BF16),
            pltpu.VMEM((D, D), BF16), pltpu.VMEM((D, D), BF16),
            pltpu.VMEM((D, D), BF16), pltpu.VMEM((D, D), BF16),
            pltpu.VMEM((D, Fd), BF16), pltpu.VMEM((Fd, D), BF16),
            pltpu.VMEM((D, 2 * D), BF16),
            pltpu.VMEM((16, 2 * D), F32),
            pltpu.VMEM((T + HALO, D), BF16),
            pltpu.VMEM((T, 2 * D), F32),
            pltpu.VMEM((T, 2 * D), BF16),
            pltpu.VMEM((8, 2 * D), F32),
            pltpu.VMEM((T + 24, D), F32),
            pltpu.VMEM((T, D), F32),
            pltpu.VMEM((T, D), BF16),
            pltpu.VMEM((2, T, D), F32),
            pltpu.VMEM((2, T, D), F32),
            pltpu.VMEM((2, T, D), F32),
            pltpu.SemaphoreType.DMA((8 + NTL,)),
            pltpu.VMEM((2, T, D), F32),
            pltpu.SemaphoreType.DMA((2,)),
        ],
        compiler_params=pltpu.CompilerParams(vmem_limit_bytes=100 * 1024 * 1024),
    )(x2, A_Lambda_re, A_Lambda_im, A_log_dt, A_Dskip,
      A_B_re, A_B_im, A_C_re, A_C_im, B_w1, B_w2, B_w3, B_w4)
    return out.reshape(1, L, D)


@jax.jit
def pallas_recurrent_scan__ssm_conv_s5__mixer_s_mlp__prompt_kernel(
    A_x, A_Lambda_re, A_Lambda_im, A_B_re, A_B_im, A_C_re, A_C_im, A_log_dt,
    A_Dskip, B_x, B_w1, B_w2, B_w3, B_w4):
    return _run(A_x, A_Lambda_re, A_Lambda_im, A_B_re, A_B_im, A_C_re, A_C_im,
                A_log_dt, A_Dskip, B_w1, B_w2, B_w3, B_w4)
```

```python
import functools
import jax
import jax.numpy as jnp
from jax import lax
import jax.experimental.pallas as pl
import jax.experimental.pallas.tpu as pltpu

F32 = jnp.float32
BF16 = jnp.bfloat16
NT_DIMS = (((1,), (1,)), ((), ()))
NSEG = 8
HALO = 16
RC = 32


def _ln(v):
    m = jnp.mean(v, axis=-1, keepdims=True)
    d = v - m
    var = jnp.mean(d * d, axis=-1, keepdims=True)
    return d * lax.rsqrt(var + 1e-5)


def _gelu(v):
    return jax.nn.gelu(v, approximate=True)


def _t8(vs):
    vs = list(vs)
    sub = lax.broadcasted_iota(jnp.int32, vs[0].shape, 0)
    for d in (4, 2, 1):
        m = (sub & d) != 0
        for a in range(8):
            if a & d:
                continue
            A, B = vs[a], vs[a + d]
            vs[a] = jnp.where(m, pltpu.roll(B, d, 0), A)
            vs[a + d] = jnp.where(m, B, pltpu.roll(A, 8 - d, 0))
    return vs


def _kernel(x_hbm, lre_ref, lim_ref, ldt_ref, dsk_ref,
            bre_hbm, bim_hbm, cre_hbm, cim_hbm, w1_hbm, w2_hbm, w3_hbm, w4_hbm,
            o_hbm,
            xv, bre, bim, cre, cim, w1, w2, w3, w4,
            cp_ref, a_ref, lx_ref, bu_ref, hb_ref, carry_ref, hext_ref, xs_ref, xp_ref,
            ys_ref, x1_ref, xd_ref, sems, obuf, osems, *, T, L, D):
    P = D
    S = T // NSEG
    NC = P // 128
    NTL = L // T

    wpairs = [(bre_hbm, bre), (bim_hbm, bim), (w1_hbm, w1), (w2_hbm, w2),
              (cre_hbm, cre), (cim_hbm, cim), (w3_hbm, w3), (w4_hbm, w4)]

    def wcopy(k):
        return pltpu.make_async_copy(wpairs[k][0], wpairs[k][1], sems.at[k])

    def xcopy(k):
        return pltpu.make_async_copy(x_hbm.at[pl.ds(k * T, T)], xv.at[pl.ds(k * T, T)],
                                     sems.at[8 + k])

    def ocopy(t):
        slot = lax.rem(t, 2)
        return pltpu.make_async_copy(obuf.at[slot], o_hbm.at[pl.ds(t * T, T)], osems.at[slot])

    def vec(r):
        return r[...].astype(F32).reshape(1, D)

    def lam_terms():
        lre = vec(lre_ref)
        lim = vec(lim_ref)
        dt = jnp.exp(vec(ldt_ref)).astype(BF16).astype(F32)
        zr = dt * lre
        zi = dt * lim
        mag = jnp.exp(zr)
        ar = mag * jnp.cos(zi)
        ai = mag * jnp.sin(zi)
        return lre, lim, ar, ai

    def init_tables():
        _, _, ar, ai = lam_terms()
        ar8 = jnp.broadcast_to(ar, (8, P))
        ai8 = jnp.broadcast_to(ai, (8, P))
        a_ref[0:8, 0:P] = ar8
        a_ref[0:8, P:2 * P] = ai8
        pr, pi = ar8, ai8
        k = 1
        while k < S:
            pr, pi = pr * pr - pi * pi, 2.0 * pr * pi
            k *= 2
        a_ref[8:16, 0:P] = pr
        a_ref[8:16, P:2 * P] = pi
        carry_ref[...] = jnp.zeros(carry_ref.shape, F32)
        hext_ref[0:8, :] = jnp.zeros((8, D), F32)

    def init_c():
        lre, lim, ar, ai = lam_terms()
        nr = ar - 1.0
        ni = ai
        den = lre * lre + lim * lim
        cr = (nr * lre + ni * lim) / den
        ci = (ni * lre - nr * lim) / den
        crev = cre[...].astype(F32)
        cimv = cim[...].astype(F32)
        cp_ref[:, 0:P] = (2.0 * (crev * cr - cimv * ci)).astype(BF16)
        cp_ref[:, P:2 * P] = (-2.0 * (crev * ci + cimv * cr)).astype(BF16)

    def stage_a0(t):
        r0 = pl.multiple_of(t * T, T)
        nstart = pl.multiple_of(jnp.minimum(r0 + T, L - HALO), HALO)
        for cidx in range(T // RC):
            xc = xv[pl.ds(r0 + cidx * RC, RC), :].astype(F32)
            xnc = _ln(xc).astype(BF16).astype(F32)
            xs_ref[cidx * RC:(cidx + 1) * RC, :] = xnc
            lx_ref[cidx * RC:(cidx + 1) * RC, :] = _ln(xnc).astype(BF16)
        xh = xv[pl.ds(nstart, HALO), :].astype(F32)
        xnhf = _ln(xh).astype(BF16).astype(F32)
        lx_ref[T:T + HALO, :] = _ln(xnhf).astype(BF16)
        for q in range(S // 8):
            for j in range(NC):
                cs = slice(128 * j, 128 * (j + 1))
                w = _t8([xs_ref[seg * S + 8 * q:seg * S + 8 * q + 8, cs] for seg in range(NSEG)])
                for k2 in range(4):
                    r = (8 * q + 2 * k2) * 8
                    xp_ref[r:r + 16, cs] = jnp.concatenate(
                        [w[2 * k2], w[2 * k2 + 1]], axis=0).astype(BF16)

    def f1(t, first):
        if first:
            wcopy(0).wait()
            wcopy(1).wait()
        xp = xp_ref[...]
        bu_ref[:, 0:P] = lax.dot_general(xp, bre[...], NT_DIMS, preferred_element_type=F32)
        bu_ref[:, P:2 * P] = lax.dot_general(xp, bim[...], NT_DIMS, preferred_element_type=F32)
        if first:
            wcopy(2).wait()
        h = _gelu(jnp.dot(lx_ref[...], w1[...], preferred_element_type=F32))
        hext_ref[8:8 + T, :] = h[0:T]
        hext_ref[8 + T:8 + T + HALO, :] = jnp.where(t < NTL - 1, h[T:T + HALO], 0.0)

    def f2():
        sub = lax.broadcasted_iota(jnp.int32, (NSEG, 128), 0)
        for j in range(NC):
            cs = slice(128 * j, 128 * (j + 1))
            ci_ = slice(P + 128 * j, P + 128 * (j + 1))
            ar8 = a_ref[0:8, cs]
            ai8 = a_ref[0:8, ci_]
            hr = bu_ref[0:8, cs]
            hi = bu_ref[0:8, ci_]
            for s in range(1, S):
                rs = slice(8 * s, 8 * (s + 1))
                br = bu_ref[rs, cs]
                bi = bu_ref[rs, ci_]
                hr, hi = ar8 * hr - ai8 * hi + br, ar8 * hi + ai8 * hr + bi
            asr = a_ref[8:9, cs]
            asi = a_ref[8:9, ci_]
            cr = carry_ref[0:1, cs]
            ci = carry_ref[0:1, ci_]
            c8r = jnp.zeros((NSEG, 128), F32)
            c8i = jnp.zeros((NSEG, 128), F32)
            for q in range(NSEG):
                c8r = jnp.where(sub == q, cr, c8r)
                c8i = jnp.where(sub == q, ci, c8i)
                cr, ci = (asr * cr - asi * ci + hr[q:q + 1, :],
                          asr * ci + asi * cr + hi[q:q + 1, :])
            carry_ref[0:1, cs] = cr
            carry_ref[0:1, ci_] = ci
            hr, hi = c8r, c8i
            for s2 in range(S // 2):
                prs, pis = [], []
                for s in (2 * s2, 2 * s2 + 1):
                    rs = slice(8 * s, 8 * (s + 1))
                    br = bu_ref[rs, cs]
                    bi = bu_ref[rs, ci_]
                    hr, hi = ar8 * hr - ai8 * hi + br, ar8 * hi + ai8 * hr + bi
                    prs.append(hr)
                    pis.append(hi)
                rs = slice(16 * s2, 16 * (s2 + 1))
                hb_ref[rs, cs] = jnp.concatenate(prs, axis=0).astype(BF16)
                hb_ref[rs, ci_] = jnp.concatenate(pis, axis=0).astype(BF16)

    def f3a(t):
        slot = lax.rem(t, 2)
        c = D // 4
        shifts = (-1, 1, -2, 2)
        cols = []
        for j in range(D // 128):
            lo, hi_ = 128 * j, 128 * (j + 1)
            g_lo, g_hi = lo // c, (hi_ - 1) // c
            a = hext_ref[pl.ds(8 + shifts[g_lo], T), lo:hi_]
            if g_hi != g_lo:
                b = hext_ref[pl.ds(8 + shifts[g_hi], T), lo:hi_]
                lane = lax.broadcasted_iota(jnp.int32, (T, 128), 1) + lo
                a = jnp.where(lane < g_hi * c, a, b)
            cols.append(a.astype(BF16))
        hsft = jnp.concatenate(cols, axis=1)
        hext_ref[0:8, :] = hext_ref[T:T + 8, :]
        xn2 = xs_ref[...]
        x1_ref[slot] = xn2 + jnp.dot(hsft, w2[...], preferred_element_type=F32)
        xd_ref[slot] = xn2 * vec(dsk_ref)

    def f3b(t):
        ys_ref[lax.rem(t, 2)] = lax.dot_general(hb_ref[...], cp_ref[...], NT_DIMS,
                                                preferred_element_type=F32)

    def b1(t):
        slot = lax.rem(t, 2)
        l1 = _ln(x1_ref[slot]).astype(BF16)
        return _gelu(jnp.dot(l1, w3[...], preferred_element_type=F32)).astype(BF16)

    def b2(t, u):
        slot = lax.rem(t, 2)
        h2 = jnp.dot(u, w4[...], preferred_element_type=F32)
        z = x1_ref[slot] + h2
        g = z * jax.nn.sigmoid(z)
        ycols = []
        for j in range(NC):
            cs = slice(128 * j, 128 * (j + 1))
            rows = [None] * (T // 8)
            for q in range(S // 8):
                w = _t8([ys_ref[slot, (8 * q + k) * 8:(8 * q + k) * 8 + 8, cs] for k in range(8)])
                for seg in range(NSEG):
                    rows[seg * (S // 8) + q] = w[seg]
            ycols.append(jnp.concatenate(rows, axis=0))
        sval = jnp.concatenate(ycols, axis=1) + xd_ref[slot]
        rp = pl.multiple_of(t * T, T)
        obuf[slot] = xv[pl.ds(rp, T), :].astype(F32) + sval * g

    xcopy(0).start()
    xcopy(1).start()
    for k in range(3):
        wcopy(k).start()
    xcopy(2).start()
    for k in range(3, 6):
        wcopy(k).start()
    xcopy(3).start()
    wcopy(6).start()
    wcopy(7).start()
    for k in range(4, NTL):
        xcopy(k).start()
    init_tables()
    xcopy(0).wait()
    xcopy(1).wait()
    stage_a0(0)
    f1(0, True)
    f2()
    wcopy(3).wait()
    xcopy(2).wait()
    f3a(0)
    stage_a0(1)
    wcopy(4).wait()
    wcopy(5).wait()
    xcopy(3).wait()
    f1(1, False)
    init_c()
    f3b(0)
    f2()
    f3a(1)
    f3b(1)
    stage_a0(2)
    wcopy(6).wait()
    wcopy(7).wait()

    def loop(i, carry):
        @pl.when(i + 2 < NTL)
        def _():
            xcopy(i + 2).wait()

        @pl.when(i >= 4)
        def _():
            ocopy(i - 4).wait()

        f1(i, False)
        u = b1(i - 2)
        f2()
        b2(i - 2, u)
        f3a(i)
        f3b(i)
        stage_a0(jnp.minimum(i + 1, NTL - 1))
        ocopy(i - 2).start()
        return carry

    lax.fori_loop(2, NTL, loop, 0)

    ocopy(NTL - 4).wait()
    ocopy(NTL - 3).wait()
    u0 = b1(NTL - 2)
    u1 = b1(NTL - 1)
    b2(NTL - 2, u0)
    ocopy(NTL - 2).start()
    b2(NTL - 1, u1)
    ocopy(NTL - 1).start()
    ocopy(NTL - 2).wait()
    ocopy(NTL - 1).wait()


def _run(A_x, A_Lambda_re, A_Lambda_im, A_B_re, A_B_im, A_C_re, A_C_im, A_log_dt,
         A_Dskip, B_w1, B_w2, B_w3, B_w4, T=256):
    _, L, D = A_x.shape
    Fd = B_w3.shape[1]
    NTL = L // T
    x2 = A_x.reshape(L, D)
    anyspec = pl.BlockSpec(memory_space=pl.ANY)
    vspec = pl.BlockSpec(memory_space=pltpu.VMEM)
    out = pl.pallas_call(
        functools.partial(_kernel, T=T, L=L, D=D),
        in_specs=[anyspec, vspec, vspec, vspec, vspec] + [anyspec] * 8,
        out_specs=anyspec,
        out_shape=jax.ShapeDtypeStruct((L, D), F32),
        scratch_shapes=[
            pltpu.VMEM((L, D), BF16),
            pltpu.VMEM((D, D), BF16), pltpu.VMEM((D, D), BF16),
            pltpu.VMEM((D, D), BF16), pltpu.VMEM((D, D), BF16),
            pltpu.VMEM((D, D), BF16), pltpu.VMEM((D, D), BF16),
            pltpu.VMEM((D, Fd), BF16), pltpu.VMEM((Fd, D), BF16),
            pltpu.VMEM((D, 2 * D), BF16),
            pltpu.VMEM((16, 2 * D), F32),
            pltpu.VMEM((T + HALO, D), BF16),
            pltpu.VMEM((T, 2 * D), F32),
            pltpu.VMEM((T, 2 * D), BF16),
            pltpu.VMEM((8, 2 * D), F32),
            pltpu.VMEM((T + 24, D), F32),
            pltpu.VMEM((T, D), F32),
            pltpu.VMEM((T, D), BF16),
            pltpu.VMEM((2, T, D), F32),
            pltpu.VMEM((2, T, D), F32),
            pltpu.VMEM((2, T, D), F32),
            pltpu.SemaphoreType.DMA((8 + NTL,)),
            pltpu.VMEM((2, T, D), F32),
            pltpu.SemaphoreType.DMA((2,)),
        ],
        compiler_params=pltpu.CompilerParams(vmem_limit_bytes=100 * 1024 * 1024),
    )(x2, A_Lambda_re, A_Lambda_im, A_log_dt, A_Dskip,
      A_B_re, A_B_im, A_C_re, A_C_im, B_w1, B_w2, B_w3, B_w4)
    return out.reshape(1, L, D)


@jax.jit
def pallas_recurrent_scan__ssm_conv_s5__mixer_s_mlp__prompt_kernel(
    A_x, A_Lambda_re, A_Lambda_im, A_B_re, A_B_im, A_C_re, A_C_im, A_log_dt,
    A_Dskip, B_x, B_w1, B_w2, B_w3, B_w4):
    return _run(A_x, A_Lambda_re, A_Lambda_im, A_B_re, A_B_im, A_C_re, A_C_im,
                A_log_dt, A_Dskip, B_w1, B_w2, B_w3, B_w4)
```

```python
import functools
import jax
import jax.numpy as jnp
from jax import lax
import jax.experimental.pallas as pl
import jax.experimental.pallas.tpu as pltpu

F32 = jnp.float32
BF16 = jnp.bfloat16
NT_DIMS = (((1,), (1,)), ((), ()))
NSEG = 8
HALO = 16
RC = 32


def _ln(v):
    m = jnp.mean(v, axis=-1, keepdims=True)
    d = v - m
    var = jnp.mean(d * d, axis=-1, keepdims=True)
    return d * lax.rsqrt(var + 1e-5)


def _gelu(v):
    return jax.nn.gelu(v, approximate=True)


def _t8(vs):
    vs = list(vs)
    sub = lax.broadcasted_iota(jnp.int32, vs[0].shape, 0)
    for d in (4, 2, 1):
        m = (sub & d) != 0
        for a in range(8):
            if a & d:
                continue
            A, B = vs[a], vs[a + d]
            vs[a] = jnp.where(m, pltpu.roll(B, d, 0), A)
            vs[a + d] = jnp.where(m, B, pltpu.roll(A, 8 - d, 0))
    return vs


def _kernel(x_hbm, lre_ref, lim_ref, ldt_ref, dsk_ref,
            bre_hbm, bim_hbm, cre_hbm, cim_hbm, w1_hbm, w2_hbm, w3_hbm, w4_hbm,
            o_hbm,
            xv, bre, bim, cre, cim, w1, w2, w3, w4,
            cp_ref, a_ref, lx_ref, bu_ref, hb_ref, carry_ref, hext_ref, xs_ref, xp_ref,
            ys_ref, x1_ref, xd_ref, sems, obuf, osems, *, T, L, D):
    P = D
    S = T // NSEG
    NC = P // 128
    NTL = L // T

    wpairs = [(bre_hbm, bre), (bim_hbm, bim), (w1_hbm, w1), (w2_hbm, w2),
              (cre_hbm, cre), (cim_hbm, cim), (w3_hbm, w3), (w4_hbm, w4)]

    def wcopy(k):
        return pltpu.make_async_copy(wpairs[k][0], wpairs[k][1], sems.at[k])

    def xcopy(k):
        return pltpu.make_async_copy(x_hbm.at[pl.ds(k * T, T)], xv.at[pl.ds(k * T, T)],
                                     sems.at[8 + k])

    def ocopy(t):
        slot = lax.rem(t, 2)
        return pltpu.make_async_copy(obuf.at[slot], o_hbm.at[pl.ds(t * T, T)], osems.at[slot])

    def vec(r):
        return r[...].astype(F32).reshape(1, D)

    def lam_terms():
        lre = vec(lre_ref)
        lim = vec(lim_ref)
        dt = jnp.exp(vec(ldt_ref)).astype(BF16).astype(F32)
        zr = dt * lre
        zi = dt * lim
        mag = jnp.exp(zr)
        ar = mag * jnp.cos(zi)
        ai = mag * jnp.sin(zi)
        return lre, lim, ar, ai

    def init_tables():
        _, _, ar, ai = lam_terms()
        ar8 = jnp.broadcast_to(ar, (8, P))
        ai8 = jnp.broadcast_to(ai, (8, P))
        a_ref[0:8, 0:P] = ar8
        a_ref[0:8, P:2 * P] = ai8
        pr, pi = ar8, ai8
        k = 1
        while k < S:
            pr, pi = pr * pr - pi * pi, 2.0 * pr * pi
            k *= 2
        a_ref[8:16, 0:P] = pr
        a_ref[8:16, P:2 * P] = pi
        carry_ref[...] = jnp.zeros(carry_ref.shape, F32)
        hext_ref[0:8, :] = jnp.zeros((8, D), F32)

    def init_c():
        lre, lim, ar, ai = lam_terms()
        nr = ar - 1.0
        ni = ai
        den = lre * lre + lim * lim
        cr = (nr * lre + ni * lim) / den
        ci = (ni * lre - nr * lim) / den
        crev = cre[...].astype(F32)
        cimv = cim[...].astype(F32)
        cp_ref[:, 0:P] = (2.0 * (crev * cr - cimv * ci)).astype(BF16)
        cp_ref[:, P:2 * P] = (-2.0 * (crev * ci + cimv * cr)).astype(BF16)

    def stage_a0(t):
        r0 = pl.multiple_of(t * T, T)
        nstart = pl.multiple_of(jnp.minimum(r0 + T, L - HALO), HALO)
        for cidx in range(T // RC):
            xc = xv[pl.ds(r0 + cidx * RC, RC), :].astype(F32)
            xnc = _ln(xc).astype(BF16).astype(F32)
            xs_ref[cidx * RC:(cidx + 1) * RC, :] = xnc
            lx_ref[cidx * RC:(cidx + 1) * RC, :] = _ln(xnc).astype(BF16)
        xh = xv[pl.ds(nstart, HALO), :].astype(F32)
        xnhf = _ln(xh).astype(BF16).astype(F32)
        lx_ref[T:T + HALO, :] = _ln(xnhf).astype(BF16)

    def f1(t, first):
        def m1():
            h = _gelu(jnp.dot(lx_ref[...], w1[...], preferred_element_type=F32))
            hext_ref[8:8 + T, :] = h[0:T]
            hext_ref[8 + T:8 + T + HALO, :] = jnp.where(t < NTL - 1, h[T:T + HALO], 0.0)

        if not first:
            m1()
        for q in range(S // 8):
            for j in range(NC):
                cs = slice(128 * j, 128 * (j + 1))
                w = _t8([xs_ref[seg * S + 8 * q:seg * S + 8 * q + 8, cs] for seg in range(NSEG)])
                for k2 in range(4):
                    r = (8 * q + 2 * k2) * 8
                    xp_ref[r:r + 16, cs] = jnp.concatenate(
                        [w[2 * k2], w[2 * k2 + 1]], axis=0).astype(BF16)
        if first:
            wcopy(0).wait()
            wcopy(1).wait()
        xp = xp_ref[...]
        bu_ref[:, 0:P] = lax.dot_general(xp, bre[...], NT_DIMS, preferred_element_type=F32)
        bu_ref[:, P:2 * P] = lax.dot_general(xp, bim[...], NT_DIMS, preferred_element_type=F32)
        if first:
            wcopy(2).wait()
            m1()

    def f2():
        sub = lax.broadcasted_iota(jnp.int32, (NSEG, 128), 0)
        for j in range(NC):
            cs = slice(128 * j, 128 * (j + 1))
            ci_ = slice(P + 128 * j, P + 128 * (j + 1))
            ar8 = a_ref[0:8, cs]
            ai8 = a_ref[0:8, ci_]
            hr = bu_ref[0:8, cs]
            hi = bu_ref[0:8, ci_]
            for s in range(1, S):
                rs = slice(8 * s, 8 * (s + 1))
                br = bu_ref[rs, cs]
                bi = bu_ref[rs, ci_]
                hr, hi = ar8 * hr - ai8 * hi + br, ar8 * hi + ai8 * hr + bi
            asr = a_ref[8:9, cs]
            asi = a_ref[8:9, ci_]
            cr = carry_ref[0:1, cs]
            ci = carry_ref[0:1, ci_]
            c8r = jnp.zeros((NSEG, 128), F32)
            c8i = jnp.zeros((NSEG, 128), F32)
            for q in range(NSEG):
                c8r = jnp.where(sub == q, cr, c8r)
                c8i = jnp.where(sub == q, ci, c8i)
                cr, ci = (asr * cr - asi * ci + hr[q:q + 1, :],
                          asr * ci + asi * cr + hi[q:q + 1, :])
            carry_ref[0:1, cs] = cr
            carry_ref[0:1, ci_] = ci
            hr, hi = c8r, c8i
            for s2 in range(S // 2):
                prs, pis = [], []
                for s in (2 * s2, 2 * s2 + 1):
                    rs = slice(8 * s, 8 * (s + 1))
                    br = bu_ref[rs, cs]
                    bi = bu_ref[rs, ci_]
                    hr, hi = ar8 * hr - ai8 * hi + br, ar8 * hi + ai8 * hr + bi
                    prs.append(hr)
                    pis.append(hi)
                rs = slice(16 * s2, 16 * (s2 + 1))
                hb_ref[rs, cs] = jnp.concatenate(prs, axis=0).astype(BF16)
                hb_ref[rs, ci_] = jnp.concatenate(pis, axis=0).astype(BF16)

    def f3a(t):
        slot = lax.rem(t, 2)
        c = D // 4
        shifts = (-1, 1, -2, 2)
        cols = []
        for j in range(D // 128):
            lo, hi_ = 128 * j, 128 * (j + 1)
            g_lo, g_hi = lo // c, (hi_ - 1) // c
            a = hext_ref[pl.ds(8 + shifts[g_lo], T), lo:hi_]
            if g_hi != g_lo:
                b = hext_ref[pl.ds(8 + shifts[g_hi], T), lo:hi_]
                lane = lax.broadcasted_iota(jnp.int32, (T, 128), 1) + lo
                a = jnp.where(lane < g_hi * c, a, b)
            cols.append(a.astype(BF16))
        hsft = jnp.concatenate(cols, axis=1)
        hext_ref[0:8, :] = hext_ref[T:T + 8, :]
        xn2 = xs_ref[...]
        x1_ref[slot] = xn2 + jnp.dot(hsft, w2[...], preferred_element_type=F32)
        xd_ref[slot] = xn2 * vec(dsk_ref)

    def f3b(t):
        ys_ref[lax.rem(t, 2)] = lax.dot_general(hb_ref[...], cp_ref[...], NT_DIMS,
                                                preferred_element_type=F32)

    def b1(t):
        slot = lax.rem(t, 2)
        l1 = _ln(x1_ref[slot]).astype(BF16)
        return _gelu(jnp.dot(l1, w3[...], preferred_element_type=F32)).astype(BF16)

    def b2(t, u):
        slot = lax.rem(t, 2)
        h2 = jnp.dot(u, w4[...], preferred_element_type=F32)
        z = x1_ref[slot] + h2
        g = z * jax.nn.sigmoid(z)
        ycols = []
        for j in range(NC):
            cs = slice(128 * j, 128 * (j + 1))
            rows = [None] * (T // 8)
            for q in range(S // 8):
                w = _t8([ys_ref[slot, (8 * q + k) * 8:(8 * q + k) * 8 + 8, cs] for k in range(8)])
                for seg in range(NSEG):
                    rows[seg * (S // 8) + q] = w[seg]
            ycols.append(jnp.concatenate(rows, axis=0))
        sval = jnp.concatenate(ycols, axis=1) + xd_ref[slot]
        rp = pl.multiple_of(t * T, T)
        obuf[slot] = xv[pl.ds(rp, T), :].astype(F32) + sval * g

    xcopy(0).start()
    xcopy(1).start()
    for k in range(3):
        wcopy(k).start()
    xcopy(2).start()
    for k in range(3, 6):
        wcopy(k).start()
    xcopy(3).start()
    wcopy(6).start()
    wcopy(7).start()
    for k in range(4, NTL):
        xcopy(k).start()
    init_tables()
    xcopy(0).wait()
    xcopy(1).wait()
    stage_a0(0)
    f1(0, True)
    f2()
    wcopy(3).wait()
    xcopy(2).wait()
    f3a(0)
    stage_a0(1)
    wcopy(4).wait()
    wcopy(5).wait()
    xcopy(3).wait()
    f1(1, False)
    init_c()
    f3b(0)
    f2()
    f3a(1)
    f3b(1)
    stage_a0(2)
    wcopy(6).wait()
    wcopy(7).wait()

    def loop(i, carry):
        @pl.when(i + 2 < NTL)
        def _():
            xcopy(i + 2).wait()

        @pl.when(i >= 4)
        def _():
            ocopy(i - 4).wait()

        f1(i, False)
        u = b1(i - 2)
        f2()
        b2(i - 2, u)
        f3a(i)
        f3b(i)
        stage_a0(jnp.minimum(i + 1, NTL - 1))
        ocopy(i - 2).start()
        return carry

    lax.fori_loop(2, NTL, loop, 0)

    ocopy(NTL - 4).wait()
    ocopy(NTL - 3).wait()
    u0 = b1(NTL - 2)
    u1 = b1(NTL - 1)
    b2(NTL - 2, u0)
    ocopy(NTL - 2).start()
    b2(NTL - 1, u1)
    ocopy(NTL - 1).start()
    ocopy(NTL - 2).wait()
    ocopy(NTL - 1).wait()


def _run(A_x, A_Lambda_re, A_Lambda_im, A_B_re, A_B_im, A_C_re, A_C_im, A_log_dt,
         A_Dskip, B_w1, B_w2, B_w3, B_w4, T=256):
    _, L, D = A_x.shape
    Fd = B_w3.shape[1]
    NTL = L // T
    x2 = A_x.reshape(L, D)
    anyspec = pl.BlockSpec(memory_space=pl.ANY)
    vspec = pl.BlockSpec(memory_space=pltpu.VMEM)
    out = pl.pallas_call(
        functools.partial(_kernel, T=T, L=L, D=D),
        in_specs=[anyspec, vspec, vspec, vspec, vspec] + [anyspec] * 8,
        out_specs=anyspec,
        out_shape=jax.ShapeDtypeStruct((L, D), F32),
        scratch_shapes=[
            pltpu.VMEM((L, D), BF16),
            pltpu.VMEM((D, D), BF16), pltpu.VMEM((D, D), BF16),
            pltpu.VMEM((D, D), BF16), pltpu.VMEM((D, D), BF16),
            pltpu.VMEM((D, D), BF16), pltpu.VMEM((D, D), BF16),
            pltpu.VMEM((D, Fd), BF16), pltpu.VMEM((Fd, D), BF16),
            pltpu.VMEM((D, 2 * D), BF16),
            pltpu.VMEM((16, 2 * D), F32),
            pltpu.VMEM((T + HALO, D), BF16),
            pltpu.VMEM((T, 2 * D), F32),
            pltpu.VMEM((T, 2 * D), BF16),
            pltpu.VMEM((8, 2 * D), F32),
            pltpu.VMEM((T + 24, D), F32),
            pltpu.VMEM((T, D), F32),
            pltpu.VMEM((T, D), BF16),
            pltpu.VMEM((2, T, D), F32),
            pltpu.VMEM((2, T, D), F32),
            pltpu.VMEM((2, T, D), F32),
            pltpu.SemaphoreType.DMA((8 + NTL,)),
            pltpu.VMEM((2, T, D), F32),
            pltpu.SemaphoreType.DMA((2,)),
        ],
        compiler_params=pltpu.CompilerParams(vmem_limit_bytes=100 * 1024 * 1024),
    )(x2, A_Lambda_re, A_Lambda_im, A_log_dt, A_Dskip,
      A_B_re, A_B_im, A_C_re, A_C_im, B_w1, B_w2, B_w3, B_w4)
    return out.reshape(1, L, D)


@jax.jit
def pallas_recurrent_scan__ssm_conv_s5__mixer_s_mlp__prompt_kernel(
    A_x, A_Lambda_re, A_Lambda_im, A_B_re, A_B_im, A_C_re, A_C_im, A_log_dt,
    A_Dskip, B_x, B_w1, B_w2, B_w3, B_w4):
    return _run(A_x, A_Lambda_re, A_Lambda_im, A_B_re, A_B_im, A_C_re, A_C_im,
                A_log_dt, A_Dskip, B_w1, B_w2, B_w3, B_w4)
```
